```python
import jax
import jax.numpy as jnp

def _softmax(x, axis=-1):
    return jax.nn.softmax(x, axis=axis)
def _gelu(x):
    return jax.nn.gelu(x, approximate=True)
def _silu(x):
    return jax.nn.silu(x)
def _sigmoid(x):
    return jax.nn.sigmoid(x)
def _layernorm(x, axis=-1, eps=1e-5):
    m = jnp.mean(x, axis=axis, keepdims=True)
    v = jnp.var(x, axis=axis, keepdims=True)
    return (x - m) / jnp.sqrt(v + eps)
def _scatter_add(tgt, idx, src, axis=0):
    return tgt.at[idx].add(src)
def _segment_sum(src, seg, n):
    return jax.ops.segment_sum(src, seg, n)
class _Rng:
    def __init__(self, key):
        self._k = key
    def _next(self):
        self._k, sub = jax.random.split(self._k)
        return sub
    def normal(self, shape):
        return jax.random.normal(self._next(), shape, dtype=jnp.bfloat16)
    def randint(self, lo, hi, shape):
        return jax.random.randint(self._next(), shape, lo, hi, dtype=jnp.int32)
    def uniform(self, shape, lo=0.0, hi=1.0):
        return jax.random.uniform(self._next(), shape, jnp.bfloat16, lo, hi)
    def permutation(self, n):
        return jax.random.permutation(self._next(), n)


kernel_name = 'standalone__structured_sparse_n_m__ragged'

def setup_inputs():
    _rng = _Rng(jax.random.key(int.from_bytes(__import__("os").urandom(4), "little")))
    _w = (lambda a: (lambda t: t.astype(jnp.bfloat16) if jnp.issubdtype(t.dtype, jnp.floating) else t)(jnp.asarray(a)))
    B, S, D = 16, 4096, 576
    assert D % 4 == 0, "d_model must be divisible by M=4 for 2:4 sparsity"
    return {
        "x": _w((lambda *s: _rng.normal(s) * 0.05)(B, S, D)),
        "w": _w((lambda *s: _rng.normal(s) * 0.05)(D, D)),
        "b": _w((lambda *s: _rng.normal(s) * 0.05)(D)),
    }

def reference(x, w, b):
    B, S, D = x.shape
    N, M = 2, 4
    G = D // M
    wg = w.reshape(G, M, D)
    mag = jnp.abs(wg)
    order = jnp.argsort(mag, 1)
    thr = jnp.take_along_axis(mag, order[:, M - N:M - N + 1, :], 1)
    mask = (lambda x, dt: x.astype(dt))(mag >= thr, w.dtype)
    wp = (wg * mask).reshape(D, D)
    return jnp.einsum("bsd,df->bsf", x, wp) + b
```

```python
import jax
import jax.numpy as jnp
from jax import lax
import jax.experimental.pallas as pl
import jax.experimental.pallas.tpu as pltpu

_T = 1.0 / 3.0
_PASSES = (
    ((1, 0, -1, 0), (({(0, 0): 1}, {(0, 0): 1, (1, 0): 1}),
                     ({(1, 5): -1}, {(4, 0): 1, (5, 0): 1}))),
    ((1, -1, 0, 0), (({(0, 1): 1, (0, 0): -1}, {(1, 0): 1}),
                     ({(0, 4): 1, (0, 5): -1}, {(5, 1): 1}))),
    ((0, 1, 0, -1), (({(1, 1): -1}, {(0, 1): 1, (1, 1): 1}),
                     ({(0, 4): 1}, {(4, 1): 1, (5, 1): 1}))),
    ((0, 0, 1, -1), (({(1, 1): 1, (1, 0): -1}, {(0, 1): 1}),
                     ({(1, 4): 1, (1, 5): -1}, {(4, 0): 1}))),
    ((0, 1, -1, 0), (({(0, 0): 1, (1, 1): 1}, {(0, 1): 1, (1, 0): -1}),
                     ({(0, 2): 1, (1, 3): -1}, {(2, 1): 1, (3, 0): 1}))),
    ((0, 0, 1, 0), (({(0, 0): 1, (1, 0): 1}, {(0, 0): 1, (0, 1): 1}),
                    ({(1, 2): 0.5, (0, 2): -1}, {(2, 0): 2, (2, 1): -1}))),
    ((0, 1, 0, 0), (({(0, 1): 1, (1, 1): 1}, {(1, 0): 1, (1, 1): 1}),
                    ({(1, 3): 0.5, (0, 3): -1}, {(3, 0): 2, (3, 1): -1}))),
    ((1, 0, 0, -1), (({(0, 6): 1, (1, 7): -1}, {(6, 0): 1, (7, 1): 1}),
                     ({(0, 4): 1, (1, 5): 1}, {(4, 0): 1, (5, 1): -1}))),
    ((0, 0, 0, 1), (({(0, 6): 0.5, (1, 6): -1}, {(6, 0): 2, (6, 1): -1}),
                    ({(0, 4): 1, (1, 4): 1}, {(4, 0): 1, (4, 1): 1}))),
    ((1, 0, 0, 0), (({(0, 7): 0.5, (1, 7): -1}, {(7, 0): 2, (7, 1): -1}),
                    ({(0, 5): 1, (1, 5): 1}, {(5, 0): 1, (5, 1): 1}))),
    ((1, 0, 2, 0), (({(1, 8): 2 * _T, (0, 8): -_T}, {(8, 0): 1}),
                    ({(0, 2): 0.5}, {(2, 0): 2, (3, 0): 1}))),
    ((2, 0, 1, 0), (({(1, 7): 0.5}, {(7, 0): 2, (6, 0): 1}),
                    ({(0, 8): 2 * _T, (1, 8): -_T}, {(8, 0): 1}))),
    ((0, 0, 1, 2), (({(1, 6): 1, (1, 7): -0.5}, {(6, 0): 1}),
                    ({(1, 2): 0.5, (1, 3): -1}, {(2, 1): 1}))),
    ((0, 1, 0, 2), (({(1, 8): 2 * _T, (0, 8): -_T}, {(8, 1): 1}),
                    ({(1, 3): 0.5}, {(2, 1): 2, (3, 1): 1}))),
    ((1, 2, 0, 0), (({(0, 7): 0.5, (0, 6): -1}, {(7, 1): 1}),
                    ({(0, 3): 1, (0, 2): -0.5}, {(3, 0): 1}))),
    ((0, 2, 0, 1), (({(0, 6): 0.5}, {(7, 1): 2, (6, 1): 1}),
                    ({(0, 8): 2 * _T, (1, 8): -_T}, {(8, 1): 1}))),
)
_KROW = (0, 128, 64, 192, 320, 448, 256, 384, 512)

_GROUP = 256
_RING = 9
_FIRST = (256, 256, 512, 1024, 2048)
_LEAD = 8


def _prune_packed(u):
    mate = lax.broadcasted_iota(jnp.int32, u.shape, 0) ^ 1
    lo = pltpu.bitcast((u << 16) & 0x7FFFFFFF, jnp.float32)
    hi = pltpu.bitcast(u & 0x7FFF0000, jnp.float32)
    big, small = jnp.maximum(lo, hi), jnp.minimum(lo, hi)
    nbig = jnp.take_along_axis(big, mate, axis=0, mode="promise_in_bounds")
    nsmall = jnp.take_along_axis(small, mate, axis=0, mode="promise_in_bounds")
    thr = jnp.maximum(jnp.minimum(big, nbig), jnp.maximum(small, nsmall))
    return u & (jnp.where(lo < thr, 0, 0xFFFF) | jnp.where(hi < thr, 0, -65536))


def _prune(w):
    u = pltpu.bitcast(w, jnp.int32)
    parts = [_prune_packed(u[8 * i:8 * i + 8]) for i in range(u.shape[0] // 8)]
    return pltpu.bitcast(jnp.concatenate(parts, axis=0), jnp.bfloat16)


def _combine(terms, get):
    acc = None
    for key, c in terms.items():
        v = get(key) if abs(c) == 1 else get(key) * abs(c)
        if acc is None:
            acc = v if c > 0 else -v
        else:
            acc = acc + v if c > 0 else acc - v
    return acc


def _kernel(x_hbm, w_hbm, b_hbm, o_hbm, xbuf, obuf, wbuf, bbuf, wt_ref, wc_ref, bb_ref,
            fsem, isem, osem, wsem):
    NB, D, S = x_hbm.shape
    F = w_hbm.shape[1]
    H = F // 2
    G = S // _GROUP
    first = [(sum(_FIRST[:j]), n) for j, n in enumerate(_FIRST)]

    def fcopy(j):
        cols = pl.ds(*first[j])
        return pltpu.make_async_copy(x_hbm.at[0, :, cols], xbuf.at[0, :, cols], fsem.at[j])

    def icopy(b):
        return pltpu.make_async_copy(x_hbm.at[b], xbuf.at[b], isem.at[b])

    def ocopy(b, slot, g):
        cols = pl.ds(g * _GROUP, _GROUP)
        return pltpu.make_async_copy(obuf.at[slot, :, cols], o_hbm.at[b, :, cols], osem.at[slot])

    def owait(slot):
        pltpu.make_async_copy(obuf.at[slot], o_hbm.at[0], osem.at[slot]).wait()

    wcopy = pltpu.make_async_copy(w_hbm, wbuf, wsem.at[0])
    bcopy = pltpu.make_async_copy(b_hbm, bbuf, wsem.at[1])
    wcopy.start()
    bcopy.start()
    for j in range(len(first)):
        fcopy(j).start(priority=1)
    for b in range(1, NB):
        icopy(b).start(priority=1)

    bcopy.wait()
    bias = bbuf[...].reshape(1, F).astype(jnp.float32)
    bb_ref[...] = jnp.broadcast_to(bias, (128, F)).T
    wcopy.wait()
    wt_ref[:, 0:512] = _prune(wbuf[0:512, :]).T.astype(jnp.float32)
    tail = _prune(wbuf[512:D, :])
    wt_ref[:, 512:640] = jnp.concatenate([tail, tail], axis=0).T.astype(jnp.float32)

    def combine_w(r, carry):
        low = lax.broadcasted_iota(jnp.int32, (48, 128), 1) < 64

        def get(key):
            i, k = key
            return wt_ref[pl.ds(pl.multiple_of(i * H + r * 48, 8), 48), pl.ds(_KROW[k] // 128 * 128, 128)]

        for p, (_, ((w0, _), (w1, _))) in enumerate(_PASSES):
            v = jnp.where(low, _combine(w0, get), _combine(w1, get)).astype(jnp.bfloat16)
            wc_ref[p, pl.ds(pl.multiple_of(r * 24, 8), 24), :] = pltpu.bitcast(v, jnp.int32)
        return carry

    lax.fori_loop(0, H // 48, combine_w, 0)

    def group(b, slot, o):
        wide = {}

        def raw(key):
            k, j = key
            return xbuf[b, pl.ds(_KROW[k], 64), pl.ds(o + j * 128, 128)]

        def get(key):
            if key not in wide:
                wide[key] = raw(key).astype(jnp.float32)
            return wide[key]

        acc = [bb_ref[pl.ds(i * H, H), :] for i in (0, 0, 1, 1)]
        for p, (coef, products) in enumerate(_PASSES):
            xs = [raw(*xt) if len(xt) == 1 else _combine(xt, get).astype(jnp.bfloat16)
                  for _, xt in products]
            m = jnp.dot(pltpu.bitcast(wc_ref[p], jnp.bfloat16), jnp.concatenate(xs, axis=0),
                        preferred_element_type=jnp.float32)
            for q, c in enumerate(coef):
                if c == -1:
                    acc[q] = acc[q] - m
                elif c:
                    acc[q] = acc[q] + (m if c == 1 else m + m)
        for q in range(4):
            obuf[slot, pl.ds(q // 2 * H, H), pl.ds(o + q % 2 * 128, 128)] = acc[q].astype(obuf.dtype)

    def wrap(s):
        return jnp.where(s >= _RING, s - _RING, s)

    def batch(b, slot):
        @pl.when(b == 0)
        def _():
            fcopy(0).wait()

        @pl.when(b > 0)
        def _():
            icopy(b).wait()

        @pl.when(b >= _RING)
        def _():
            owait(slot)

        done = [jnp.clip(2 * b - NB + d, 0, NB - 1) for d in range(3)]
        for g in range(G):
            for j in range(1, len(first)):
                if first[j][0] == g * _GROUP:
                    @pl.when(b == 0)
                    def _():
                        fcopy(j).wait()
            group(b, slot, g * _GROUP)
            for q in (_LEAD + 2 * g, _LEAD + 2 * g + 1):
                ready = b >= (NB // 2 - 1 if q >= 2 * G else NB // 2)
                if q - G > g:
                    ready = jnp.logical_and(ready, b < NB - 1)

                @pl.when(ready)
                def _():
                    ocopy(done[q // G], wrap(done[q // G]), q % G).start()
        return wrap(slot + 1)

    lax.fori_loop(0, NB, batch, 0)
    for g in range(G):
        for q in (_LEAD + 2 * g, _LEAD + 2 * g + 1):
            if g < q - G < G:
                ocopy(NB - 1, (NB - 1) % _RING, q - G).start()
    for b in range(NB - _RING, NB):
        owait(b % _RING)


@jax.jit
def pallas_standalone__structured_sparse_n_m__ragged_kernel(
    x: jax.Array,
    w: jax.Array,
    b: jax.Array,
):
    B, S, D = x.shape
    F = w.shape[1]
    xt = jnp.transpose(x, (0, 2, 1))
    out = pl.pallas_call(
        _kernel,
        in_specs=[pl.BlockSpec(memory_space=pl.ANY)] * 3,
        out_specs=pl.BlockSpec(memory_space=pl.ANY),
        out_shape=jax.ShapeDtypeStruct((B, F, S), x.dtype),
        scratch_shapes=[
            pltpu.VMEM((B, D, S), x.dtype),
            pltpu.VMEM((_RING, F, S), x.dtype),
            pltpu.VMEM((D, F), w.dtype),
            pltpu.VMEM((F,), b.dtype),
            pltpu.VMEM((F, 640), jnp.float32),
            pltpu.VMEM((len(_PASSES), F // 4, 128), jnp.int32),
            pltpu.VMEM((F, 128), jnp.float32),
            pltpu.SemaphoreType.DMA((len(_FIRST),)),
            pltpu.SemaphoreType.DMA((B,)),
            pltpu.SemaphoreType.DMA((_RING,)),
            pltpu.SemaphoreType.DMA((2,)),
        ],
        compiler_params=pltpu.CompilerParams(
            vmem_limit_bytes=124 * 1024 * 1024,
            disable_bounds_checks=True,
            disable_semaphore_checks=True,
            flags={"XLA_TPU_RESCHEDULE_DMA_DONES": True},
        ),
    )(xt, w, b)
    return jnp.transpose(out, (0, 2, 1))
```

```python
import jax
import jax.numpy as jnp
from jax import lax
import jax.experimental.pallas as pl
import jax.experimental.pallas.tpu as pltpu

_T = 1.0 / 3.0
_PASSES = (
    ((0, 0, 1, -1), (({(1, 1): 1, (1, 0): -1}, {(0, 1): 1}),
                     ({(1, 4): 1, (1, 5): -1}, {(4, 0): 1}))),
    ((1, -1, 0, 0), (({(0, 1): 1, (0, 0): -1}, {(1, 0): 1}),
                     ({(0, 4): 1, (0, 5): -1}, {(5, 1): 1}))),
    ((0, 0, 1, 2), (({(1, 6): 1, (1, 7): -0.5}, {(6, 0): 1}),
                    ({(1, 2): 0.5, (1, 3): -1}, {(2, 1): 1}))),
    ((1, 2, 0, 0), (({(0, 7): 0.5, (0, 6): -1}, {(7, 1): 1}),
                    ({(0, 3): 1, (0, 2): -0.5}, {(3, 0): 1}))),
    ((1, 0, -1, 0), (({(0, 0): 1}, {(0, 0): 1, (1, 0): 1}),
                     ({(1, 5): -1}, {(4, 0): 1, (5, 0): 1}))),
    ((1, 0, 2, 0), (({(1, 8): 2 * _T, (0, 8): -_T}, {(8, 0): 1}),
                    ({(0, 2): 0.5}, {(2, 0): 2, (3, 0): 1}))),
    ((0, 1, 0, -1), (({(1, 1): -1}, {(0, 1): 1, (1, 1): 1}),
                     ({(0, 4): 1}, {(4, 1): 1, (5, 1): 1}))),
    ((0, 1, 0, 2), (({(1, 8): 2 * _T, (0, 8): -_T}, {(8, 1): 1}),
                    ({(1, 3): 0.5}, {(2, 1): 2, (3, 1): 1}))),
    ((0, 1, -1, 0), (({(0, 0): 1, (1, 1): 1}, {(0, 1): 1, (1, 0): -1}),
                     ({(0, 2): 1, (1, 3): -1}, {(2, 1): 1, (3, 0): 1}))),
    ((1, 0, 0, -1), (({(0, 6): 1, (1, 7): -1}, {(6, 0): 1, (7, 1): 1}),
                     ({(0, 4): 1, (1, 5): 1}, {(4, 0): 1, (5, 1): -1}))),
    ((0, 2, 0, 1), (({(0, 6): 0.5}, {(7, 1): 2, (6, 1): 1}),
                    ({(0, 8): 2 * _T, (1, 8): -_T}, {(8, 1): 1}))),
    ((2, 0, 1, 0), (({(1, 7): 0.5}, {(7, 0): 2, (6, 0): 1}),
                    ({(0, 8): 2 * _T, (1, 8): -_T}, {(8, 0): 1}))),
    ((0, 0, 1, 0), (({(0, 0): 1, (1, 0): 1}, {(0, 0): 1, (0, 1): 1}),
                    ({(1, 2): 0.5, (0, 2): -1}, {(2, 0): 2, (2, 1): -1}))),
    ((0, 1, 0, 0), (({(0, 1): 1, (1, 1): 1}, {(1, 0): 1, (1, 1): 1}),
                    ({(1, 3): 0.5, (0, 3): -1}, {(3, 0): 2, (3, 1): -1}))),
    ((0, 0, 0, 1), (({(0, 6): 0.5, (1, 6): -1}, {(6, 0): 2, (6, 1): -1}),
                    ({(0, 4): 1, (1, 4): 1}, {(4, 0): 1, (4, 1): 1}))),
    ((1, 0, 0, 0), (({(0, 7): 0.5, (1, 7): -1}, {(7, 0): 2, (7, 1): -1}),
                    ({(0, 5): 1, (1, 5): 1}, {(5, 0): 1, (5, 1): 1}))),
)
_KROW = (0, 128, 64, 192, 320, 448, 256, 384, 512)

_GROUP = 256
_FIRST = (256, 256, 512, 1024, 2048)
_OCOLS = 1024
_LEAD = 16
_TAIL = ((0, 2048), (2048, 1024))


def _prune_packed(u):
    mate = lax.broadcasted_iota(jnp.int32, u.shape, 0) ^ 1
    lo = pltpu.bitcast((u << 16) & 0x7FFFFFFF, jnp.float32)
    hi = pltpu.bitcast(u & 0x7FFF0000, jnp.float32)
    big, small = jnp.maximum(lo, hi), jnp.minimum(lo, hi)
    nbig = jnp.take_along_axis(big, mate, axis=0, mode="promise_in_bounds")
    nsmall = jnp.take_along_axis(small, mate, axis=0, mode="promise_in_bounds")
    thr = jnp.maximum(jnp.minimum(big, nbig), jnp.maximum(small, nsmall))
    return u & (jnp.where(lo < thr, 0, 0xFFFF) | jnp.where(hi < thr, 0, -65536))


def _prune(w):
    u = pltpu.bitcast(w, jnp.int32)
    parts = [_prune_packed(u[8 * i:8 * i + 8]) for i in range(u.shape[0] // 8)]
    return pltpu.bitcast(jnp.concatenate(parts, axis=0), jnp.bfloat16)


def _combine(terms, get):
    acc = None
    for key, c in terms.items():
        v = get(key) if abs(c) == 1 else get(key) * abs(c)
        if acc is None:
            acc = v if c > 0 else -v
        else:
            acc = acc + v if c > 0 else acc - v
    return acc


def _kernel(x_hbm, w_hbm, b_hbm, o_hbm, xbuf, obuf, wbuf, bbuf, wt_ref, wc_ref, bb_ref,
            fsem, isem, osem, wsem):
    _, D, S = x_hbm.shape
    F = w_hbm.shape[1]
    H = F // 2
    NP = o_hbm.shape[0]
    RING = obuf.shape[0]
    G = 2 * S // _GROUP
    NC = S // _OCOLS
    NQ = 128 // 8 * NC
    first = [(sum(_FIRST[:j]), n) for j, n in enumerate(_FIRST)]

    def fcopy(h, j):
        cols = pl.ds(*first[j])
        return pltpu.make_async_copy(x_hbm.at[h, :, cols], xbuf.at[h, :, cols], fsem.at[2 * j + h])

    def icopy(m):
        pair = pl.ds(2 * m, 2)
        return pltpu.make_async_copy(x_hbm.at[pair], xbuf.at[pair], isem.at[m])

    def ostart(m, slot, *block):
        block = tuple(pl.ds(*b) for b in block)
        pltpu.make_async_copy(obuf.at[(slot,) + block], o_hbm.at[(m,) + block], osem.at[slot]).start()

    def streams(r, c):
        return (0, 9), (8 * r, 8), (c, _OCOLS)

    def owait(slot):
        pltpu.make_async_copy(obuf.at[slot], obuf.at[slot], osem.at[slot]).wait()

    tail, pending = [], []
    for g in range(G):
        c = g // 2 * _GROUP
        for c0, n in _TAIL:
            if g % 2 and c + _GROUP == c0 + n:
                pending += [streams(r, cc) for r in range(16) for cc in range(c0, c0 + n, _OCOLS)]
        if c >= sum(_TAIL[-1]):
            rows = (((4, 1), (64, 64)), ((5, 4), (0, 128))) if g % 2 else (((0, 4), (0, 128)), ((4, 1), (0, 64)))
            pending += [r + ((c, _GROUP),) for r in rows]
        n = 8 if g < G - 1 else len(pending)
        tail.append(pending[:n])
        pending = pending[n:]

    wcopy = pltpu.make_async_copy(w_hbm, wbuf, wsem.at[0])
    bcopy = pltpu.make_async_copy(b_hbm, bbuf, wsem.at[1])
    wcopy.start()
    bcopy.start()
    for j in range(len(first)):
        lax.fori_loop(0, 2, lambda h, _: fcopy(h, j).start(priority=1), None)
    lax.fori_loop(1, NP, lambda m, _: icopy(m).start(priority=1), None)

    bcopy.wait()
    bias = bbuf[...].reshape(1, F).astype(jnp.float32)
    bb_ref[...] = jnp.broadcast_to(bias, (128, F)).T
    wcopy.wait()
    wt_ref[:, 0:512] = _prune(wbuf[0:512, :]).T.astype(jnp.float32)
    last = _prune(wbuf[512:D, :])
    wt_ref[:, 512:640] = jnp.concatenate([last, last], axis=0).T.astype(jnp.float32)

    def combine_w(r, carry):
        low = lax.broadcasted_iota(jnp.int32, (48, 128), 1) < 64

        def get(key):
            i, k = key
            return wt_ref[pl.ds(pl.multiple_of(i * H + r * 48, 8), 48), pl.ds(_KROW[k] // 128 * 128, 128)]

        for p, (_, ((w0, _), (w1, _))) in enumerate(_PASSES):
            v = jnp.where(low, _combine(w0, get), _combine(w1, get)).astype(jnp.bfloat16)
            wc_ref[p, pl.ds(pl.multiple_of(r * 24, 8), 24), :] = pltpu.bitcast(v, jnp.int32)
        return carry

    lax.fori_loop(0, H // 48, combine_w, 0)

    def group(m, slot, h, o):
        wide = {}

        def raw(key):
            k, j = key
            return xbuf[2 * m + h, pl.ds(_KROW[k], 64), pl.ds(o + j * 128, 128)]

        def get(key):
            if key not in wide:
                wide[key] = raw(key).astype(jnp.float32)
            return wide[key]

        acc = [bb_ref[pl.ds(i * H, H), :] for i in (0, 0, 1, 1)]
        for p, (coef, products) in enumerate(_PASSES):
            xs = [raw(*xt) if len(xt) == 1 else _combine(xt, get).astype(jnp.bfloat16)
                  for _, xt in products]
            y = jnp.dot(pltpu.bitcast(wc_ref[p], jnp.bfloat16), jnp.concatenate(xs, axis=0),
                        preferred_element_type=jnp.float32)
            for q, c in enumerate(coef):
                if c == -1:
                    acc[q] = acc[q] - y
                elif c:
                    acc[q] = acc[q] + (y if c == 1 else y + y)
        for q in range(4):
            out = acc[q].astype(obuf.dtype)
            r0 = h * F + q // 2 * H
            cuts = sorted({r0, r0 + H} | set(range(pl.cdiv(r0, 128) * 128, r0 + H, 128)))
            for lo, hi in zip(cuts[:-1], cuts[1:]):
                obuf[slot, lo // 128, pl.ds(lo % 128, hi - lo), pl.ds(o + q % 2 * 128, 128)] = (
                    out[lo - r0:hi - r0])

    def wrap(s):
        return jnp.where(s >= RING, s - RING, s)

    def pair(m, slot):
        @pl.when(m > 0)
        def _():
            icopy(m).wait()

        @pl.when(m >= RING)
        def _():
            owait(slot)

        def last_only(n, block):
            pl.when(m == NP - 1)(lambda: ostart(n, n % RING, *block))

        done = [jnp.clip(2 * m - NP + d, 0, NP - 1) for d in range(3)]
        for g in range(G):
            h, o = g % 2, g // 2 * _GROUP
            for j in range(len(first)):
                if first[j][0] == o:
                    pl.when(m == 0)(lambda: fcopy(h, j).wait())
            if g == 0:
                for q in range(_LEAD):
                    last_only(NP - 2, streams(q // NC, q % NC * _OCOLS))
            group(m, slot, h, o)
            for e in range(2 * NQ // G):
                d, q = divmod(_LEAD + 2 * NQ // G * g + e, NQ)
                ready = jnp.logical_and(m >= NP // 2 - d // 2, m < NP - d)
                pl.when(ready)(lambda: ostart(done[d], wrap(done[d]), *streams(q // NC, q % NC * _OCOLS)))
            for block in tail[g]:
                last_only(NP - 1, block)
        return wrap(slot + 1)

    lax.fori_loop(0, NP, pair, 0)
    for m in range(NP - RING, NP):
        owait(m % RING)


@jax.jit
def pallas_standalone__structured_sparse_n_m__ragged_kernel(
    x: jax.Array,
    w: jax.Array,
    b: jax.Array,
):
    B, S, D = x.shape
    F = w.shape[1]
    xt = jnp.transpose(x, (0, 2, 1))
    out = pl.pallas_call(
        _kernel,
        in_specs=[pl.BlockSpec(memory_space=pl.ANY)] * 3,
        out_specs=pl.BlockSpec(memory_space=pl.ANY),
        out_shape=jax.ShapeDtypeStruct((B // 2, 2 * F // 128, 128, S), x.dtype),
        scratch_shapes=[
            pltpu.VMEM((B, D, S), x.dtype),
            pltpu.VMEM((B // 4 + 1, 2 * F // 128, 128, S), x.dtype),
            pltpu.VMEM((D, F), w.dtype),
            pltpu.VMEM((F,), b.dtype),
            pltpu.VMEM((F, 640), jnp.float32),
            pltpu.VMEM((len(_PASSES), F // 4, 128), jnp.int32),
            pltpu.VMEM((F, 128), jnp.float32),
            pltpu.SemaphoreType.DMA((2 * len(_FIRST),)),
            pltpu.SemaphoreType.DMA((B // 2,)),
            pltpu.SemaphoreType.DMA((B // 4 + 1,)),
            pltpu.SemaphoreType.DMA((2,)),
        ],
        compiler_params=pltpu.CompilerParams(
            vmem_limit_bytes=127 * 1024 * 1024,
            disable_bounds_checks=True,
            disable_semaphore_checks=True,
            flags={"XLA_TPU_RESCHEDULE_DMA_DONES": True},
        ),
    )(xt, w, b)
    return jnp.transpose(out.reshape(B, F, S), (0, 2, 1))
```

```python
import jax
import jax.numpy as jnp
from jax import lax
import jax.experimental.pallas as pl
import jax.experimental.pallas.tpu as pltpu

_T = 1.0 / 3.0
_PASSES = (
    ((0, 0, 1, -1), (({(1, 1): 1, (1, 0): -1}, {(0, 1): 1}),
                     ({(1, 4): 1, (1, 5): -1}, {(4, 0): 1}))),
    ((1, -1, 0, 0), (({(0, 1): 1, (0, 0): -1}, {(1, 0): 1}),
                     ({(0, 4): 1, (0, 5): -1}, {(5, 1): 1}))),
    ((0, 0, 1, 2), (({(1, 6): 1, (1, 7): -0.5}, {(6, 0): 1}),
                    ({(1, 2): 0.5, (1, 3): -1}, {(2, 1): 1}))),
    ((1, 2, 0, 0), (({(0, 7): 0.5, (0, 6): -1}, {(7, 1): 1}),
                    ({(0, 3): 1, (0, 2): -0.5}, {(3, 0): 1}))),
    ((1, 0, -1, 0), (({(0, 0): 1}, {(0, 0): 1, (1, 0): 1}),
                     ({(1, 5): -1}, {(4, 0): 1, (5, 0): 1}))),
    ((1, 0, 2, 0), (({(1, 8): 2 * _T, (0, 8): -_T}, {(8, 0): 1}),
                    ({(0, 2): 0.5}, {(2, 0): 2, (3, 0): 1}))),
    ((0, 1, 0, -1), (({(1, 1): -1}, {(0, 1): 1, (1, 1): 1}),
                     ({(0, 4): 1}, {(4, 1): 1, (5, 1): 1}))),
    ((0, 1, 0, 2), (({(1, 8): 2 * _T, (0, 8): -_T}, {(8, 1): 1}),
                    ({(1, 3): 0.5}, {(2, 1): 2, (3, 1): 1}))),
    ((0, 1, -1, 0), (({(0, 0): 1, (1, 1): 1}, {(0, 1): 1, (1, 0): -1}),
                     ({(0, 2): 1, (1, 3): -1}, {(2, 1): 1, (3, 0): 1}))),
    ((1, 0, 0, -1), (({(0, 6): 1, (1, 7): -1}, {(6, 0): 1, (7, 1): 1}),
                     ({(0, 4): 1, (1, 5): 1}, {(4, 0): 1, (5, 1): -1}))),
    ((0, 2, 0, 1), (({(0, 6): 0.5}, {(7, 1): 2, (6, 1): 1}),
                    ({(0, 8): 2 * _T, (1, 8): -_T}, {(8, 1): 1}))),
    ((2, 0, 1, 0), (({(1, 7): 0.5}, {(7, 0): 2, (6, 0): 1}),
                    ({(0, 8): 2 * _T, (1, 8): -_T}, {(8, 0): 1}))),
    ((0, 0, 1, 0), (({(0, 0): 1, (1, 0): 1}, {(0, 0): 1, (0, 1): 1}),
                    ({(1, 2): 0.5, (0, 2): -1}, {(2, 0): 2, (2, 1): -1}))),
    ((0, 1, 0, 0), (({(0, 1): 1, (1, 1): 1}, {(1, 0): 1, (1, 1): 1}),
                    ({(1, 3): 0.5, (0, 3): -1}, {(3, 0): 2, (3, 1): -1}))),
    ((0, 0, 0, 1), (({(0, 6): 0.5, (1, 6): -1}, {(6, 0): 2, (6, 1): -1}),
                    ({(0, 4): 1, (1, 4): 1}, {(4, 0): 1, (4, 1): 1}))),
    ((1, 0, 0, 0), (({(0, 7): 0.5, (1, 7): -1}, {(7, 0): 2, (7, 1): -1}),
                    ({(0, 5): 1, (1, 5): 1}, {(5, 0): 1, (5, 1): 1}))),
)
_KROW = (0, 128, 64, 192, 320, 448, 256, 384, 512)

_GROUP = 256
_FIRST = (256, 256, 512, 1024, 2048)
_OCOLS = 1024
_LEAD = 12
_START = 30
_TAIL = ((0, 2048), (2048, 1024))


def _prune_packed(u):
    mate = lax.broadcasted_iota(jnp.int32, u.shape, 0) ^ 1
    lo = pltpu.bitcast((u << 16) & 0x7FFFFFFF, jnp.float32)
    hi = pltpu.bitcast(u & 0x7FFF0000, jnp.float32)
    big, small = jnp.maximum(lo, hi), jnp.minimum(lo, hi)
    nbig = jnp.take_along_axis(big, mate, axis=0, mode="promise_in_bounds")
    nsmall = jnp.take_along_axis(small, mate, axis=0, mode="promise_in_bounds")
    thr = jnp.maximum(jnp.minimum(big, nbig), jnp.maximum(small, nsmall))
    return u & (jnp.where(lo < thr, 0, 0xFFFF) | jnp.where(hi < thr, 0, -65536))


def _prune(w):
    u = pltpu.bitcast(w, jnp.int32)
    parts = [_prune_packed(u[8 * i:8 * i + 8]) for i in range(u.shape[0] // 8)]
    return pltpu.bitcast(jnp.concatenate(parts, axis=0), jnp.bfloat16)


def _combine(terms, get):
    acc = None
    for key, c in terms.items():
        v = get(key) if abs(c) == 1 else get(key) * abs(c)
        if acc is None:
            acc = v if c > 0 else -v
        else:
            acc = acc + v if c > 0 else acc - v
    return acc


def _kernel(x_hbm, w_hbm, b_hbm, o_hbm, xbuf, obuf, wbuf, bbuf, wt_ref, wc_ref, bb_ref,
            acc_ref, fsem, isem, osem, wsem):
    _, D, S = x_hbm.shape
    F = w_hbm.shape[1]
    H = F // 2
    NP = o_hbm.shape[0]
    RING = obuf.shape[0]
    G = 2 * S // _GROUP
    NC = S // _OCOLS
    NQ = 128 // 8 * NC
    QG = 2 * NQ // G
    first = [(sum(_FIRST[:j]), n) for j, n in enumerate(_FIRST)]

    def fcopy(h, j):
        cols = pl.ds(*first[j])
        return pltpu.make_async_copy(x_hbm.at[h, :, cols], xbuf.at[h, :, cols], fsem.at[2 * j + h])

    def icopy(m):
        pair = pl.ds(2 * m, 2)
        return pltpu.make_async_copy(x_hbm.at[pair], xbuf.at[pair], isem.at[m])

    def ostart(m, slot, *block):
        block = tuple(pl.ds(*b) for b in block)
        pltpu.make_async_copy(obuf.at[(slot,) + block], o_hbm.at[(m,) + block], osem.at[slot]).start()

    def streams(r, c):
        return (0, 9), (8 * r, 8), (c, _OCOLS)

    def regular(q):
        return streams(q // NC, q % NC * _OCOLS)

    def owait(slot):
        pltpu.make_async_copy(obuf.at[slot], obuf.at[slot], osem.at[slot]).wait()

    tail, pending = [], []
    for g in range(G):
        c = g // 2 * _GROUP
        for c0, n in _TAIL:
            if g % 2 and c + _GROUP == c0 + n:
                pending += [streams(r, cc) for r in range(16) for cc in range(c0, c0 + n, _OCOLS)]
        if c >= sum(_TAIL[-1]):
            rows = (((4, 1), (64, 64)), ((5, 4), (0, 128))) if g % 2 else (((0, 4), (0, 128)), ((4, 1), (0, 64)))
            pending += [r + ((c, _GROUP),) for r in rows]
        n = 8 if g < G - 1 else len(pending)
        tail.append(pending[:n])
        pending = pending[n:]

    def wcopy(j):
        rows = pl.ds(128 * j, min(128, D - 128 * j))
        return pltpu.make_async_copy(w_hbm.at[rows], wbuf.at[rows], wsem.at[j])

    NW = wt_ref.shape[0]
    bcopy = pltpu.make_async_copy(b_hbm, bbuf, wsem.at[NW])
    bcopy.start()
    for j in range(NW):
        wcopy(j).start()
    for j in range(len(first)):
        lax.fori_loop(0, 2, lambda h, _: fcopy(h, j).start(), None)
    lax.fori_loop(1, NP, lambda m, _: icopy(m).start(), None)

    bcopy.wait()
    bias = bbuf[...].reshape(1, F).astype(jnp.float32)
    bb_ref[...] = jnp.broadcast_to(bias, (128, F)).T
    low = lax.broadcasted_iota(jnp.int32, (16, 128), 1) < 64
    for j in range(NW):
        wcopy(j).wait()
        wp = _prune(wbuf[128 * j:min(128 * j + 128, D), :])
        if wp.shape[0] < 128:
            wp = jnp.concatenate([wp, wp], axis=0)
        wt_ref[j] = pltpu.bitcast(wp.T, jnp.int32)
        for r in range(H // 16):
            wide = {}

            def get(key):
                key = key[0], _KROW[key[1]] // 128
                if key not in wide:
                    u = wt_ref[key[1], pl.ds(key[0] * H // 2 + 8 * r, 8), :]
                    wide[key] = pltpu.bitcast(u, jnp.bfloat16).astype(jnp.float32)
                return wide[key]

            for p, (_, ((w0, _), (w1, _))) in enumerate(_PASSES):
                if max(_KROW[k] // 128 for _, k in (*w0, *w1)) == j:
                    v = jnp.where(low, _combine(w0, get), _combine(w1, get))
                    wc_ref[p, pl.ds(16 * r, 16), :] = v.astype(wc_ref.dtype)
    wc_words = wc_ref.bitcast(jnp.int32)

    def group(m, slot, h, o):
        wide = {}

        def raw(key):
            k, j = key
            return xbuf[2 * m + h, pl.ds(_KROW[k], 64), pl.ds(o + j * 128, 128)]

        def get(key):
            if key not in wide:
                wide[key] = raw(key).astype(jnp.float32)
            return wide[key]

        acc = [bb_ref[pl.ds(i * H, H), :] for i in (0, 0, 1, 1)]
        for p, (coef, products) in enumerate(_PASSES):
            if p and p % 4 == 0:
                for q in range(4):
                    acc_ref[q] = acc[q]
                acc = [acc_ref[q] for q in range(4)]
                wide.clear()
            if all(len(xt) == 1 for _, xt in products):
                xs = jnp.concatenate([raw(*xt) for _, xt in products], axis=0)
            else:
                xs = jnp.concatenate([_combine(xt, get) for _, xt in products], axis=0)
            y = jnp.dot(pltpu.bitcast(wc_words[p], jnp.bfloat16), xs.astype(jnp.bfloat16),
                        preferred_element_type=jnp.float32)
            for q, c in enumerate(coef):
                if c == -1:
                    acc[q] = acc[q] - y
                elif c:
                    acc[q] = acc[q] + (y if c == 1 else y + y)
        for q in range(4):
            out = acc[q].astype(obuf.dtype)
            r0 = h * F + q // 2 * H
            cuts = sorted({r0, r0 + H} | set(range(pl.cdiv(r0, 128) * 128, r0 + H, 128)))
            for lo, hi in zip(cuts[:-1], cuts[1:]):
                obuf[slot, lo // 128, pl.ds(lo % 128, hi - lo), pl.ds(o + q % 2 * 128, 128)] = (
                    out[lo - r0:hi - r0])

    def wrap(s):
        return jnp.where(s >= RING, s - RING, s)

    def pair(m, slot):
        @pl.when(m > 0)
        def _():
            icopy(m).wait()

        @pl.when(m >= RING)
        def _():
            owait(slot)

        def only_at(step, n, block):
            pl.when(m == step)(lambda: ostart(n, n % RING, *block))

        done = [jnp.clip(2 * m - NP + d, 0, NP - 1) for d in range(3)]
        for g in range(G):
            h, o = g % 2, g // 2 * _GROUP
            for j in range(len(first)):
                if first[j][0] == o:
                    pl.when(m == 0)(lambda: fcopy(h, j).wait())
            if g == 0:
                for q in range(_LEAD):
                    only_at(NP - 1, NP - 2, regular(q))
            group(m, slot, h, o)
            for q in range(_LEAD):
                if g == max(_START, G - pl.cdiv(_LEAD - q, QG)):
                    only_at(NP // 2 - 1, 0, regular(q))
            for e in range(QG):
                d, q = divmod(_LEAD + QG * g + e, NQ)
                complete = jnp.logical_and(m >= NP // 2, m < NP - d)
                pl.when(complete)(lambda: ostart(done[d], wrap(done[d]), *regular(q)))
            for block in tail[g]:
                only_at(NP - 1, NP - 1, block)
        return wrap(slot + 1)

    lax.fori_loop(0, NP, pair, 0)
    for m in range(NP - RING, NP):
        owait(m % RING)


@jax.jit
def pallas_standalone__structured_sparse_n_m__ragged_kernel(
    x: jax.Array,
    w: jax.Array,
    b: jax.Array,
):
    B, S, D = x.shape
    F = w.shape[1]
    xt = jnp.transpose(x, (0, 2, 1))
    out = pl.pallas_call(
        _kernel,
        in_specs=[pl.BlockSpec(memory_space=pl.ANY)] * 3,
        out_specs=pl.BlockSpec(memory_space=pl.ANY),
        out_shape=jax.ShapeDtypeStruct((B // 2, 2 * F // 128, 128, S), x.dtype),
        scratch_shapes=[
            pltpu.VMEM((B, D, S), x.dtype),
            pltpu.VMEM((B // 4 + 1, 2 * F // 128, 128, S), x.dtype),
            pltpu.VMEM((D, F), w.dtype),
            pltpu.VMEM((F,), b.dtype),
            pltpu.VMEM((pl.cdiv(D, 128), F // 2, 128), jnp.int32),
            pltpu.VMEM((len(_PASSES), F // 2, 128), jnp.bfloat16),
            pltpu.VMEM((F, 128), jnp.float32),
            pltpu.VMEM((4, F // 2, 128), jnp.float32),
            pltpu.SemaphoreType.DMA((2 * len(_FIRST),)),
            pltpu.SemaphoreType.DMA((B // 2,)),
            pltpu.SemaphoreType.DMA((B // 4 + 1,)),
            pltpu.SemaphoreType.DMA((pl.cdiv(D, 128) + 1,)),
        ],
        compiler_params=pltpu.CompilerParams(
            vmem_limit_bytes=127 * 1024 * 1024,
            disable_bounds_checks=True,
            disable_semaphore_checks=True,
            flags={"XLA_TPU_RESCHEDULE_DMA_DONES": True},
        ),
    )(xt, w, b)
    return jnp.transpose(out.reshape(B, F, S), (0, 2, 1))
```

```python
import jax
import jax.numpy as jnp
from jax import lax
import jax.experimental.pallas as pl
import jax.experimental.pallas.tpu as pltpu

_T = 1.0 / 3.0
_PASSES = (
    ((0, 0, 1, -1), (({(1, 1): 1, (1, 0): -1}, {(0, 1): 1}),
                     ({(1, 4): 1, (1, 5): -1}, {(4, 0): 1}))),
    ((1, -1, 0, 0), (({(0, 1): 1, (0, 0): -1}, {(1, 0): 1}),
                     ({(0, 4): 1, (0, 5): -1}, {(5, 1): 1}))),
    ((0, 0, 1, 2), (({(1, 6): 1, (1, 7): -0.5}, {(6, 0): 1}),
                    ({(1, 2): 0.5, (1, 3): -1}, {(2, 1): 1}))),
    ((1, 2, 0, 0), (({(0, 7): 0.5, (0, 6): -1}, {(7, 1): 1}),
                    ({(0, 3): 1, (0, 2): -0.5}, {(3, 0): 1}))),
    ((1, 0, -1, 0), (({(0, 0): 1}, {(0, 0): 1, (1, 0): 1}),
                     ({(1, 5): -1}, {(4, 0): 1, (5, 0): 1}))),
    ((1, 0, 2, 0), (({(1, 8): 2 * _T, (0, 8): -_T}, {(8, 0): 1}),
                    ({(0, 2): 0.5}, {(2, 0): 2, (3, 0): 1}))),
    ((0, 1, 0, -1), (({(1, 1): -1}, {(0, 1): 1, (1, 1): 1}),
                     ({(0, 4): 1}, {(4, 1): 1, (5, 1): 1}))),
    ((0, 1, 0, 2), (({(1, 8): 2 * _T, (0, 8): -_T}, {(8, 1): 1}),
                    ({(1, 3): 0.5}, {(2, 1): 2, (3, 1): 1}))),
    ((0, 1, -1, 0), (({(0, 0): 1, (1, 1): 1}, {(0, 1): 1, (1, 0): -1}),
                     ({(0, 2): 1, (1, 3): -1}, {(2, 1): 1, (3, 0): 1}))),
    ((1, 0, 0, -1), (({(0, 6): 1, (1, 7): -1}, {(6, 0): 1, (7, 1): 1}),
                     ({(0, 4): 1, (1, 5): 1}, {(4, 0): 1, (5, 1): -1}))),
    ((0, 2, 0, 1), (({(0, 6): 0.5}, {(7, 1): 2, (6, 1): 1}),
                    ({(0, 8): 2 * _T, (1, 8): -_T}, {(8, 1): 1}))),
    ((2, 0, 1, 0), (({(1, 7): 0.5}, {(7, 0): 2, (6, 0): 1}),
                    ({(0, 8): 2 * _T, (1, 8): -_T}, {(8, 0): 1}))),
    ((0, 0, 1, 0), (({(0, 0): 1, (1, 0): 1}, {(0, 0): 1, (0, 1): 1}),
                    ({(1, 2): 0.5, (0, 2): -1}, {(2, 0): 2, (2, 1): -1}))),
    ((0, 1, 0, 0), (({(0, 1): 1, (1, 1): 1}, {(1, 0): 1, (1, 1): 1}),
                    ({(1, 3): 0.5, (0, 3): -1}, {(3, 0): 2, (3, 1): -1}))),
    ((0, 0, 0, 1), (({(0, 6): 0.5, (1, 6): -1}, {(6, 0): 2, (6, 1): -1}),
                    ({(0, 4): 1, (1, 4): 1}, {(4, 0): 1, (4, 1): 1}))),
    ((1, 0, 0, 0), (({(0, 7): 0.5, (1, 7): -1}, {(7, 0): 2, (7, 1): -1}),
                    ({(0, 5): 1, (1, 5): 1}, {(5, 0): 1, (5, 1): 1}))),
)
_KROW = (0, 128, 64, 192, 320, 448, 256, 384, 512)

_GROUP = 256
_FIRST = (256, 256, 512, 1024, 2048)
_OCOLS = 1024
_LEAD = 12
_START = 30
_TAIL = ((0, 2048), (2048, 1024))


def _prune_packed(u):
    mate = lax.broadcasted_iota(jnp.int32, u.shape, 0) ^ 1
    lo = pltpu.bitcast((u << 16) & 0x7FFFFFFF, jnp.float32)
    hi = pltpu.bitcast(u & 0x7FFF0000, jnp.float32)
    big, small = jnp.maximum(lo, hi), jnp.minimum(lo, hi)
    nbig = jnp.take_along_axis(big, mate, axis=0, mode="promise_in_bounds")
    nsmall = jnp.take_along_axis(small, mate, axis=0, mode="promise_in_bounds")
    thr = jnp.maximum(jnp.minimum(big, nbig), jnp.maximum(small, nsmall))
    return u & (jnp.where(lo < thr, 0, 0xFFFF) | jnp.where(hi < thr, 0, -65536))


def _prune(w):
    u = pltpu.bitcast(w, jnp.int32)
    parts = [_prune_packed(u[8 * i:8 * i + 8]) for i in range(u.shape[0] // 8)]
    return pltpu.bitcast(jnp.concatenate(parts, axis=0), jnp.bfloat16)


def _max_exponent(u):
    lo = pltpu.bitcast((u << 16) & 0x7F800000, jnp.float32)
    hi = pltpu.bitcast(u & 0x7F800000, jnp.float32)
    return pltpu.bitcast(jnp.max(jnp.maximum(lo, hi), axis=0, keepdims=True), jnp.int32)


def _combine(terms, get):
    acc = None
    for key, c in terms.items():
        v = get(key) if abs(c) == 1 else get(key) * abs(c)
        if acc is None:
            acc = v if c > 0 else -v
        else:
            acc = acc + v if c > 0 else acc - v
    return acc


def _kernel(x_hbm, w_hbm, b_hbm, o_hbm, xbuf, obuf, wbuf, bbuf, wt_ref, wc_ref, bb_ref,
            xs_ref, acc_ref, fsem, isem, osem, wsem):
    _, D, S = x_hbm.shape
    F = w_hbm.shape[1]
    H = F // 2
    NP = o_hbm.shape[0]
    RING = obuf.shape[0]
    G = 2 * S // _GROUP
    NC = S // _OCOLS
    NQ = 128 // 8 * NC
    QG = 2 * NQ // G
    first = [(sum(_FIRST[:j]), n) for j, n in enumerate(_FIRST)]

    def fcopy(h, j):
        cols = pl.ds(*first[j])
        return pltpu.make_async_copy(x_hbm.at[h, :, cols], xbuf.at[h, :, cols], fsem.at[2 * j + h])

    def icopy(m):
        pair = pl.ds(2 * m, 2)
        return pltpu.make_async_copy(x_hbm.at[pair], xbuf.at[pair], isem.at[m])

    def ostart(m, slot, *block):
        block = tuple(pl.ds(*b) for b in block)
        pltpu.make_async_copy(obuf.at[(slot,) + block], o_hbm.at[(m,) + block], osem.at[slot]).start()

    def streams(r, c):
        return (0, 9), (8 * r, 8), (c, _OCOLS)

    def regular(q):
        return streams(q // NC, q % NC * _OCOLS)

    def owait(slot):
        pltpu.make_async_copy(obuf.at[slot], obuf.at[slot], osem.at[slot]).wait()

    tail, pending = [], []
    for g in range(G):
        c = g // 2 * _GROUP
        for c0, n in _TAIL:
            if g % 2 and c + _GROUP == c0 + n:
                pending += [streams(r, cc) for r in range(16) for cc in range(c0, c0 + n, _OCOLS)]
        if c >= sum(_TAIL[-1]):
            rows = (((4, 1), (64, 64)), ((5, 4), (0, 128))) if g % 2 else (((0, 4), (0, 128)), ((4, 1), (0, 64)))
            pending += [r + ((c, _GROUP),) for r in rows]
        n = 8 if g < G - 1 else len(pending)
        tail.append(pending[:n])
        pending = pending[n:]

    def wcopy(j):
        rows = pl.ds(128 * j, min(128, D - 128 * j))
        return pltpu.make_async_copy(w_hbm.at[rows], wbuf.at[rows], wsem.at[j])

    NW = wt_ref.shape[0]
    bcopy = pltpu.make_async_copy(b_hbm, bbuf, wsem.at[NW])
    bcopy.start()
    for j in range(NW):
        wcopy(j).start()
    for j in range(len(first)):
        lax.fori_loop(0, 2, lambda h, _: fcopy(h, j).start(), None)
    lax.fori_loop(1, NP, lambda m, _: icopy(m).start(), None)

    bcopy.wait()
    bias = bbuf[...].reshape(1, F).astype(jnp.float32)
    bb_ref[...] = jnp.broadcast_to(bias, (128, F)).T
    low = lax.broadcasted_iota(jnp.int32, (16, 128), 1) < 64
    expo, down, up = {}, {}, {}
    for j in range(NW):
        wcopy(j).wait()
        wp = _prune(wbuf[128 * j:min(128 * j + 128, D), :])
        if wp.shape[0] < 128:
            wp = jnp.concatenate([wp, wp], axis=0)
        wt = pltpu.bitcast(wp.T, jnp.int32)
        wt_ref[j] = wt
        if j < NW - 1:
            expo[j] = _max_exponent(wt)
            if j % 2 == 0:
                continue
            for t in (j - 1, j):
                shift = jnp.maximum(expo[t] - jnp.maximum(expo[j - 1], expo[j]), -64 << 23)
                down[t] = pltpu.bitcast((127 << 23) + shift, jnp.float32)
                up[t] = pltpu.bitcast((127 << 23) - shift, jnp.float32)
                xs_ref[pl.ds(128 * t, 128), :] = jnp.broadcast_to(down[t], (128, 128)).T
        for r in range(H // 16):
            wide = {}

            def get(key):
                i, t = key[0], _KROW[key[1]] // 128
                if (i, t) not in wide:
                    u = wt_ref[t, pl.ds(i * H // 2 + 8 * r, 8), :]
                    v = pltpu.bitcast(u, jnp.bfloat16).astype(jnp.float32)
                    wide[i, t] = v * up[t] if t in up else v
                return wide[i, t]

            for p, (_, ((w0, x0), (w1, x1))) in enumerate(_PASSES):
                if max(_KROW[k] // 128 | (k < 8) for _, k in (*w0, *w1)) == j:
                    v = jnp.where(low, _combine(w0, get), _combine(w1, get))
                    if len(x0) == len(x1) == 1:
                        t0, t1 = (_KROW[k] // 128 for k, _ in (*x0, *x1))
                        v = v * jnp.where(low, down[t0], down[t1])
                    wc_ref[p, pl.ds(16 * r, 16), :] = v.astype(wc_ref.dtype)
    wc_words = wc_ref.bitcast(jnp.int32)

    def group(m, slot, h, o):
        wide = {}

        def raw(key):
            k, j = key
            return xbuf[2 * m + h, pl.ds(_KROW[k], 64), pl.ds(o + j * 128, 128)]

        def get(key):
            if key not in wide:
                v = raw(key).astype(jnp.float32)
                wide[key] = v * xs_ref[pl.ds(_KROW[key[0]], 64), :] if key[0] < 8 else v
            return wide[key]

        acc = [bb_ref[pl.ds(i * H, H), :] for i in (0, 0, 1, 1)]
        for p, (coef, products) in enumerate(_PASSES):
            if p and p % 4 == 0:
                for q in range(4):
                    acc_ref[q] = acc[q]
                acc = [acc_ref[q] for q in range(4)]
                wide.clear()
            if all(len(xt) == 1 for _, xt in products):
                xs = jnp.concatenate([raw(*xt) for _, xt in products], axis=0)
            else:
                xs = jnp.concatenate([_combine(xt, get) for _, xt in products], axis=0)
            y = jnp.dot(pltpu.bitcast(wc_words[p], jnp.bfloat16), xs.astype(jnp.bfloat16),
                        preferred_element_type=jnp.float32)
            for q, c in enumerate(coef):
                if c == -1:
                    acc[q] = acc[q] - y
                elif c:
                    acc[q] = acc[q] + (y if c == 1 else y + y)
        for q in range(4):
            out = acc[q].astype(obuf.dtype)
            r0 = h * F + q // 2 * H
            cuts = sorted({r0, r0 + H} | set(range(pl.cdiv(r0, 128) * 128, r0 + H, 128)))
            for lo, hi in zip(cuts[:-1], cuts[1:]):
                obuf[slot, lo // 128, pl.ds(lo % 128, hi - lo), pl.ds(o + q % 2 * 128, 128)] = (
                    out[lo - r0:hi - r0])

    def wrap(s):
        return jnp.where(s >= RING, s - RING, s)

    def pair(m, slot):
        @pl.when(m > 0)
        def _():
            icopy(m).wait()

        @pl.when(m >= RING)
        def _():
            owait(slot)

        def only_at(step, n, block):
            pl.when(m == step)(lambda: ostart(n, n % RING, *block))

        done = [jnp.clip(2 * m - NP + d, 0, NP - 1) for d in range(3)]
        for g in range(G):
            h, o = g % 2, g // 2 * _GROUP
            for j in range(len(first)):
                if first[j][0] == o:
                    pl.when(m == 0)(lambda: fcopy(h, j).wait())
            if g == 0:
                for q in range(_LEAD):
                    only_at(NP - 1, NP - 2, regular(q))
            group(m, slot, h, o)
            for q in range(_LEAD):
                if g == max(_START, G - pl.cdiv(_LEAD - q, QG)):
                    only_at(NP // 2 - 1, 0, regular(q))
            for e in range(QG):
                d, q = divmod(_LEAD + QG * g + e, NQ)
                complete = jnp.logical_and(m >= NP // 2, m < NP - d)
                pl.when(complete)(lambda: ostart(done[d], wrap(done[d]), *regular(q)))
            for block in tail[g]:
                only_at(NP - 1, NP - 1, block)
        return wrap(slot + 1)

    lax.fori_loop(0, NP, pair, 0)
    for m in range(NP - RING, NP):
        owait(m % RING)


@jax.jit
def pallas_standalone__structured_sparse_n_m__ragged_kernel(
    x: jax.Array,
    w: jax.Array,
    b: jax.Array,
):
    B, S, D = x.shape
    F = w.shape[1]
    xt = jnp.transpose(x, (0, 2, 1))
    out = pl.pallas_call(
        _kernel,
        in_specs=[pl.BlockSpec(memory_space=pl.ANY)] * 3,
        out_specs=pl.BlockSpec(memory_space=pl.ANY),
        out_shape=jax.ShapeDtypeStruct((B // 2, 2 * F // 128, 128, S), x.dtype),
        scratch_shapes=[
            pltpu.VMEM((B, D, S), x.dtype),
            pltpu.VMEM((B // 4 + 1, 2 * F // 128, 128, S), x.dtype),
            pltpu.VMEM((D, F), w.dtype),
            pltpu.VMEM((F,), b.dtype),
            pltpu.VMEM((pl.cdiv(D, 128), F // 2, 128), jnp.int32),
            pltpu.VMEM((len(_PASSES), F // 2, 128), jnp.bfloat16),
            pltpu.VMEM((F, 128), jnp.float32),
            pltpu.VMEM((D // 128 * 128, 128), jnp.float32),
            pltpu.VMEM((4, F // 2, 128), jnp.float32),
            pltpu.SemaphoreType.DMA((2 * len(_FIRST),)),
            pltpu.SemaphoreType.DMA((B // 2,)),
            pltpu.SemaphoreType.DMA((B // 4 + 1,)),
            pltpu.SemaphoreType.DMA((pl.cdiv(D, 128) + 1,)),
        ],
        compiler_params=pltpu.CompilerParams(
            vmem_limit_bytes=127 * 1024 * 1024,
            disable_bounds_checks=True,
            disable_semaphore_checks=True,
            flags={"XLA_TPU_RESCHEDULE_DMA_DONES": True},
        ),
    )(xt, w, b)
    return jnp.transpose(out.reshape(B, F, S), (0, 2, 1))
```

```python
import jax
import jax.numpy as jnp
from jax import lax
import jax.experimental.pallas as pl
import jax.experimental.pallas.tpu as pltpu

_T = 1.0 / 3.0
_PASSES = (
    ((0, 0, 1, -1), (({(1, 1): 1, (1, 0): -1}, {(0, 1): 1}),
                     ({(1, 4): 1, (1, 5): -1}, {(4, 0): 1}))),
    ((1, -1, 0, 0), (({(0, 1): 1, (0, 0): -1}, {(1, 0): 1}),
                     ({(0, 4): 1, (0, 5): -1}, {(5, 1): 1}))),
    ((0, 0, 1, 2), (({(1, 6): 1, (1, 7): -0.5}, {(6, 0): 1}),
                    ({(1, 2): 0.5, (1, 3): -1}, {(2, 1): 1}))),
    ((1, 2, 0, 0), (({(0, 7): 0.5, (0, 6): -1}, {(7, 1): 1}),
                    ({(0, 3): 1, (0, 2): -0.5}, {(3, 0): 1}))),
    ((1, 0, -1, 0), (({(0, 0): 1}, {(0, 0): 1, (1, 0): 1}),
                     ({(1, 5): -1}, {(4, 0): 1, (5, 0): 1}))),
    ((1, 0, 2, 0), (({(1, 8): 2 * _T, (0, 8): -_T}, {(8, 0): 1}),
                    ({(0, 2): 0.5}, {(2, 0): 2, (3, 0): 1}))),
    ((0, 1, 0, -1), (({(1, 1): -1}, {(0, 1): 1, (1, 1): 1}),
                     ({(0, 4): 1}, {(4, 1): 1, (5, 1): 1}))),
    ((0, 1, 0, 2), (({(1, 8): 2 * _T, (0, 8): -_T}, {(8, 1): 1}),
                    ({(1, 3): 0.5}, {(2, 1): 2, (3, 1): 1}))),
    ((0, 1, -1, 0), (({(0, 0): 1, (1, 1): 1}, {(0, 1): 1, (1, 0): -1}),
                     ({(0, 2): 1, (1, 3): -1}, {(2, 1): 1, (3, 0): 1}))),
    ((1, 0, 0, -1), (({(0, 6): 1, (1, 7): -1}, {(6, 0): 1, (7, 1): 1}),
                     ({(0, 4): 1, (1, 5): 1}, {(4, 0): 1, (5, 1): -1}))),
    ((0, 2, 0, 1), (({(0, 6): 0.5}, {(7, 1): 2, (6, 1): 1}),
                    ({(0, 8): 2 * _T, (1, 8): -_T}, {(8, 1): 1}))),
    ((2, 0, 1, 0), (({(1, 7): 0.5}, {(7, 0): 2, (6, 0): 1}),
                    ({(0, 8): 2 * _T, (1, 8): -_T}, {(8, 0): 1}))),
    ((0, 0, 1, 0), (({(0, 0): 1, (1, 0): 1}, {(0, 0): 1, (0, 1): 1}),
                    ({(1, 2): 0.5, (0, 2): -1}, {(2, 0): 2, (2, 1): -1}))),
    ((0, 1, 0, 0), (({(0, 1): 1, (1, 1): 1}, {(1, 0): 1, (1, 1): 1}),
                    ({(1, 3): 0.5, (0, 3): -1}, {(3, 0): 2, (3, 1): -1}))),
    ((0, 0, 0, 1), (({(0, 6): 0.5, (1, 6): -1}, {(6, 0): 2, (6, 1): -1}),
                    ({(0, 4): 1, (1, 4): 1}, {(4, 0): 1, (4, 1): 1}))),
    ((1, 0, 0, 0), (({(0, 7): 0.5, (1, 7): -1}, {(7, 0): 2, (7, 1): -1}),
                    ({(0, 5): 1, (1, 5): 1}, {(5, 0): 1, (5, 1): 1}))),
)
_KROW = (0, 128, 64, 192, 320, 448, 256, 384, 512)

_GROUP = 256
_FIRST = (256, 256, 512, 1024, 2048)
_OCOLS = 1024
_LEAD = 12
_START = 30
_NEXT = 4
_TAIL = ((0, 2048), (2048, 1024))


def _prune_packed(u):
    mate = lax.broadcasted_iota(jnp.int32, u.shape, 0) ^ 1
    lo = pltpu.bitcast((u << 16) & 0x7FFFFFFF, jnp.float32)
    hi = pltpu.bitcast(u & 0x7FFF0000, jnp.float32)
    big, small = jnp.maximum(lo, hi), jnp.minimum(lo, hi)
    nbig = jnp.take_along_axis(big, mate, axis=0, mode="promise_in_bounds")
    nsmall = jnp.take_along_axis(small, mate, axis=0, mode="promise_in_bounds")
    thr = jnp.maximum(jnp.minimum(big, nbig), jnp.maximum(small, nsmall))
    return u & (jnp.where(lo < thr, 0, 0xFFFF) | jnp.where(hi < thr, 0, -65536))


def _prune(w):
    u = pltpu.bitcast(w, jnp.int32)
    parts = [_prune_packed(u[8 * i:8 * i + 8]) for i in range(u.shape[0] // 8)]
    return pltpu.bitcast(jnp.concatenate(parts, axis=0), jnp.bfloat16)


def _max_exponent(u):
    lo = pltpu.bitcast((u << 16) & 0x7F800000, jnp.float32)
    hi = pltpu.bitcast(u & 0x7F800000, jnp.float32)
    return pltpu.bitcast(jnp.max(jnp.maximum(lo, hi), axis=0, keepdims=True), jnp.int32)


def _combine(terms, get):
    acc = None
    for key, c in terms.items():
        v = get(key) if abs(c) == 1 else get(key) * abs(c)
        if acc is None:
            acc = v if c > 0 else -v
        else:
            acc = acc + v if c > 0 else acc - v
    return acc


def _kernel(x_hbm, w_hbm, b_hbm, o_hbm, xbuf, obuf, wbuf, bbuf, wt_ref, wc_ref, bb_ref,
            xs_ref, acc_ref, fsem, isem, osem, wsem):
    _, D, S = x_hbm.shape
    F = w_hbm.shape[1]
    H = F // 2
    NP = o_hbm.shape[0]
    RING = obuf.shape[0]
    G = 2 * S // _GROUP
    NC = S // _OCOLS
    NQ = 128 // 8 * NC
    QG = 2 * NQ // G
    first = [(sum(_FIRST[:j]), n) for j, n in enumerate(_FIRST)]

    def fcopy(h, j):
        cols = pl.ds(*first[j])
        return pltpu.make_async_copy(x_hbm.at[h, :, cols], xbuf.at[h, :, cols], fsem.at[2 * j + h])

    def icopy(m):
        pair = pl.ds(2 * m, 2)
        return pltpu.make_async_copy(x_hbm.at[pair], xbuf.at[pair], isem.at[m])

    def ostart(m, slot, *block):
        block = tuple(pl.ds(*b) for b in block)
        pltpu.make_async_copy(obuf.at[(slot,) + block], o_hbm.at[(m,) + block], osem.at[slot]).start()

    def streams(r, c):
        return (0, 9), (8 * r, 8), (c, _OCOLS)

    def regular(q):
        return streams(q // NC, q % NC * _OCOLS)

    def owait(slot):
        pltpu.make_async_copy(obuf.at[slot], obuf.at[slot], osem.at[slot]).wait()

    tail, pending = [], []
    for g in range(G):
        c = g // 2 * _GROUP
        for c0, n in _TAIL:
            if g % 2 and c + _GROUP == c0 + n:
                pending += [streams(r, cc) for r in range(16) for cc in range(c0, c0 + n, _OCOLS)]
        if c >= sum(_TAIL[-1]):
            rows = (((4, 1), (64, 64)), ((5, 4), (0, 128))) if g % 2 else (((0, 4), (0, 128)), ((4, 1), (0, 64)))
            pending += [r + ((c, _GROUP),) for r in rows]
        n = 8 if g < G - 1 else len(pending)
        tail.append(pending[:n])
        pending = pending[n:]

    def wcopy(j):
        rows = pl.ds(128 * j, min(128, D - 128 * j))
        return pltpu.make_async_copy(w_hbm.at[rows], wbuf.at[rows], wsem.at[j])

    NW = wt_ref.shape[0]
    bcopy = pltpu.make_async_copy(b_hbm, bbuf, wsem.at[NW])
    bcopy.start()
    for j in range(NW):
        wcopy(j).start()
    for j in range(len(first)):
        lax.fori_loop(0, 2, lambda h, _: fcopy(h, j).start(), None)
    lax.fori_loop(1, NP, lambda m, _: icopy(m).start(), None)

    bcopy.wait()
    bias = bbuf[...].reshape(1, F).astype(jnp.float32)
    bb_ref[...] = jnp.broadcast_to(bias, (128, F)).T
    low = lax.broadcasted_iota(jnp.int32, (16, 128), 1) < 64
    expo, down, up = {}, {}, {}
    for j in range(NW):
        wcopy(j).wait()
        wp = _prune(wbuf[128 * j:min(128 * j + 128, D), :])
        if wp.shape[0] < 128:
            wp = jnp.concatenate([wp, wp], axis=0)
        wt = pltpu.bitcast(wp.T, jnp.int32)
        wt_ref[j] = wt
        if j < NW - 1:
            expo[j] = _max_exponent(wt)
            if j % 2 == 0:
                continue
            for t in (j - 1, j):
                shift = jnp.maximum(expo[t] - jnp.maximum(expo[j - 1], expo[j]), -64 << 23)
                down[t] = pltpu.bitcast((127 << 23) + shift, jnp.float32)
                up[t] = pltpu.bitcast((127 << 23) - shift, jnp.float32)
                xs_ref[pl.ds(128 * t, 128), :] = jnp.broadcast_to(down[t], (128, 128)).T
        for r in range(H // 16):
            wide = {}

            def get(key):
                i, t = key[0], _KROW[key[1]] // 128
                if (i, t) not in wide:
                    u = wt_ref[t, pl.ds(i * H // 2 + 8 * r, 8), :]
                    v = pltpu.bitcast(u, jnp.bfloat16).astype(jnp.float32)
                    wide[i, t] = v * up[t] if t in up else v
                return wide[i, t]

            for p, (_, ((w0, x0), (w1, x1))) in enumerate(_PASSES):
                if max(_KROW[k] // 128 | (k < 8) for _, k in (*w0, *w1)) == j:
                    v = jnp.where(low, _combine(w0, get), _combine(w1, get))
                    if len(x0) == len(x1) == 1:
                        t0, t1 = (_KROW[k] // 128 for k, _ in (*x0, *x1))
                        v = v * jnp.where(low, down[t0], down[t1])
                    wc_ref[p, pl.ds(16 * r, 16), :] = v.astype(wc_ref.dtype)
    wc_words = wc_ref.bitcast(jnp.int32)

    def group(m, slot, h, o):
        wide = {}

        def raw(key):
            k, j = key
            return xbuf[2 * m + h, pl.ds(_KROW[k], 64), pl.ds(o + j * 128, 128)]

        def get(key):
            if key not in wide:
                v = raw(key).astype(jnp.float32)
                wide[key] = v * xs_ref[pl.ds(_KROW[key[0]], 64), :] if key[0] < 8 else v
            return wide[key]

        acc = [bb_ref[pl.ds(i * H, H), :] for i in (0, 0, 1, 1)]
        for p, (coef, products) in enumerate(_PASSES):
            if p and p % 4 == 0:
                for q in range(4):
                    acc_ref[q] = acc[q]
                acc = [acc_ref[q] for q in range(4)]
                wide.clear()
            if all(len(xt) == 1 for _, xt in products):
                xs = jnp.concatenate([raw(*xt) for _, xt in products], axis=0)
            else:
                xs = jnp.concatenate([_combine(xt, get) for _, xt in products], axis=0)
            y = jnp.dot(pltpu.bitcast(wc_words[p], jnp.bfloat16), xs.astype(jnp.bfloat16),
                        preferred_element_type=jnp.float32)
            for q, c in enumerate(coef):
                if c == -1:
                    acc[q] = acc[q] - y
                elif c:
                    acc[q] = acc[q] + (y if c == 1 else y + y)
        for q in range(4):
            out = acc[q].astype(obuf.dtype)
            r0 = h * F + q // 2 * H
            cuts = sorted({r0, r0 + H} | set(range(pl.cdiv(r0, 128) * 128, r0 + H, 128)))
            for lo, hi in zip(cuts[:-1], cuts[1:]):
                obuf[slot, lo // 128, pl.ds(lo % 128, hi - lo), pl.ds(o + q % 2 * 128, 128)] = (
                    out[lo - r0:hi - r0])

    def wrap(s):
        return jnp.where(s >= RING, s - RING, s)

    def pair(m, slot):
        @pl.when(m > 0)
        def _():
            icopy(m).wait()

        @pl.when(m >= RING)
        def _():
            owait(slot)

        def only_at(step, n, block):
            pl.when(m == step)(lambda: ostart(n, n % RING, *block))

        done = [jnp.clip(2 * m - NP + d, 0, NP - 1) for d in range(3)]
        for g in range(G):
            h, o = g % 2, g // 2 * _GROUP
            for j in range(len(first)):
                if first[j][0] == o:
                    pl.when(m == 0)(lambda: fcopy(h, j).wait())
            if g == 0:
                for q in range(_NEXT, _LEAD):
                    only_at(NP - 1, NP - 2, regular(q))
            group(m, slot, h, o)
            for q in range(_LEAD):
                if g == max(_START, G - pl.cdiv(_LEAD - q, QG)):
                    only_at(NP // 2 - 1, 0, regular(q))
            for e in range(QG):
                d, q = divmod(_LEAD + QG * g + e, NQ)
                complete = jnp.logical_and(m >= NP // 2, m < NP - d)
                pl.when(complete)(lambda: ostart(done[d], wrap(done[d]), *regular(q)))
            for block in tail[g]:
                only_at(NP - 1, NP - 1, block)
        for q in range(_NEXT):
            only_at(NP - 2, NP - 2, regular(q))
        return wrap(slot + 1)

    lax.fori_loop(0, NP, pair, 0)
    for m in range(NP - RING, NP):
        owait(m % RING)


@jax.jit
def pallas_standalone__structured_sparse_n_m__ragged_kernel(
    x: jax.Array,
    w: jax.Array,
    b: jax.Array,
):
    B, S, D = x.shape
    F = w.shape[1]
    xt = jnp.transpose(x, (0, 2, 1))
    out = pl.pallas_call(
        _kernel,
        in_specs=[pl.BlockSpec(memory_space=pl.ANY)] * 3,
        out_specs=pl.BlockSpec(memory_space=pl.ANY),
        out_shape=jax.ShapeDtypeStruct((B // 2, 2 * F // 128, 128, S), x.dtype),
        scratch_shapes=[
            pltpu.VMEM((B, D, S), x.dtype),
            pltpu.VMEM((B // 4 + 1, 2 * F // 128, 128, S), x.dtype),
            pltpu.VMEM((D, F), w.dtype),
            pltpu.VMEM((F,), b.dtype),
            pltpu.VMEM((pl.cdiv(D, 128), F // 2, 128), jnp.int32),
            pltpu.VMEM((len(_PASSES), F // 2, 128), jnp.bfloat16),
            pltpu.VMEM((F, 128), jnp.float32),
            pltpu.VMEM((D // 128 * 128, 128), jnp.float32),
            pltpu.VMEM((4, F // 2, 128), jnp.float32),
            pltpu.SemaphoreType.DMA((2 * len(_FIRST),)),
            pltpu.SemaphoreType.DMA((B // 2,)),
            pltpu.SemaphoreType.DMA((B // 4 + 1,)),
            pltpu.SemaphoreType.DMA((pl.cdiv(D, 128) + 1,)),
        ],
        compiler_params=pltpu.CompilerParams(
            vmem_limit_bytes=127 * 1024 * 1024,
            disable_bounds_checks=True,
            disable_semaphore_checks=True,
            flags={"XLA_TPU_RESCHEDULE_DMA_DONES": True},
        ),
    )(xt, w, b)
    return jnp.transpose(out.reshape(B, F, S), (0, 2, 1))
```

```python
import jax
import jax.numpy as jnp
from jax import lax
import jax.experimental.pallas as pl
import jax.experimental.pallas.tpu as pltpu

_T = 1.0 / 3.0
_PASSES = (
    ((0, 0, 1, -1), (({(1, 1): 1, (1, 0): -1}, {(0, 1): 1}),
                     ({(1, 4): 1, (1, 5): -1}, {(4, 0): 1}))),
    ((1, -1, 0, 0), (({(0, 1): 1, (0, 0): -1}, {(1, 0): 1}),
                     ({(0, 4): 1, (0, 5): -1}, {(5, 1): 1}))),
    ((0, 0, 1, 2), (({(1, 6): 1, (1, 7): -0.5}, {(6, 0): 1}),
                    ({(1, 2): 0.5, (1, 3): -1}, {(2, 1): 1}))),
    ((1, 2, 0, 0), (({(0, 7): 0.5, (0, 6): -1}, {(7, 1): 1}),
                    ({(0, 3): 1, (0, 2): -0.5}, {(3, 0): 1}))),
    ((1, 0, -1, 0), (({(0, 0): 1}, {(0, 0): 1, (1, 0): 1}),
                     ({(1, 5): -1}, {(4, 0): 1, (5, 0): 1}))),
    ((1, 0, 2, 0), (({(1, 8): 2 * _T, (0, 8): -_T}, {(8, 0): 1}),
                    ({(0, 2): 0.5}, {(2, 0): 2, (3, 0): 1}))),
    ((0, 1, 0, -1), (({(1, 1): -1}, {(0, 1): 1, (1, 1): 1}),
                     ({(0, 4): 1}, {(4, 1): 1, (5, 1): 1}))),
    ((0, 1, 0, 2), (({(1, 8): 2 * _T, (0, 8): -_T}, {(8, 1): 1}),
                    ({(1, 3): 0.5}, {(2, 1): 2, (3, 1): 1}))),
    ((0, 1, -1, 0), (({(0, 0): 1, (1, 1): 1}, {(0, 1): 1, (1, 0): -1}),
                     ({(0, 2): 1, (1, 3): -1}, {(2, 1): 1, (3, 0): 1}))),
    ((1, 0, 0, -1), (({(0, 6): 1, (1, 7): -1}, {(6, 0): 1, (7, 1): 1}),
                     ({(0, 4): 1, (1, 5): 1}, {(4, 0): 1, (5, 1): -1}))),
    ((0, 2, 0, 1), (({(0, 6): 0.5}, {(7, 1): 2, (6, 1): 1}),
                    ({(0, 8): 2 * _T, (1, 8): -_T}, {(8, 1): 1}))),
    ((2, 0, 1, 0), (({(1, 7): 0.5}, {(7, 0): 2, (6, 0): 1}),
                    ({(0, 8): 2 * _T, (1, 8): -_T}, {(8, 0): 1}))),
    ((0, 0, 1, 0), (({(0, 0): 1, (1, 0): 1}, {(0, 0): 1, (0, 1): 1}),
                    ({(1, 2): 0.5, (0, 2): -1}, {(2, 0): 2, (2, 1): -1}))),
    ((0, 1, 0, 0), (({(0, 1): 1, (1, 1): 1}, {(1, 0): 1, (1, 1): 1}),
                    ({(1, 3): 0.5, (0, 3): -1}, {(3, 0): 2, (3, 1): -1}))),
    ((0, 0, 0, 1), (({(0, 6): 0.5, (1, 6): -1}, {(6, 0): 2, (6, 1): -1}),
                    ({(0, 4): 1, (1, 4): 1}, {(4, 0): 1, (4, 1): 1}))),
    ((1, 0, 0, 0), (({(0, 7): 0.5, (1, 7): -1}, {(7, 0): 2, (7, 1): -1}),
                    ({(0, 5): 1, (1, 5): 1}, {(5, 0): 1, (5, 1): 1}))),
)
_KROW = (0, 128, 64, 192, 320, 448, 256, 384, 512)

_GROUP = 256
_FIRST = (256, 256, 512, 512, 512, 2048)
_OCOLS = 1024
_LEAD = 16
_START = 30
_TAIL = ((0, 2048), (2048, 1024))


def _prune_packed(u):
    mate = lax.broadcasted_iota(jnp.int32, u.shape, 0) ^ 1
    lo = pltpu.bitcast((u << 16) & 0x7FFFFFFF, jnp.float32)
    hi = pltpu.bitcast(u & 0x7FFF0000, jnp.float32)
    big, small = jnp.maximum(lo, hi), jnp.minimum(lo, hi)
    nbig = jnp.take_along_axis(big, mate, axis=0, mode="promise_in_bounds")
    nsmall = jnp.take_along_axis(small, mate, axis=0, mode="promise_in_bounds")
    thr = jnp.maximum(jnp.minimum(big, nbig), jnp.maximum(small, nsmall))
    return u & (jnp.where(lo < thr, 0, 0xFFFF) | jnp.where(hi < thr, 0, -65536))


def _prune(w):
    u = pltpu.bitcast(w, jnp.int32)
    parts = [_prune_packed(u[8 * i:8 * i + 8]) for i in range(u.shape[0] // 8)]
    return pltpu.bitcast(jnp.concatenate(parts, axis=0), jnp.bfloat16)


def _max_exponent(u):
    mag = u & 0x7F807F80
    top = jnp.maximum(pltpu.bitcast(mag << 16, jnp.float32), pltpu.bitcast(mag, jnp.float32))
    return pltpu.bitcast(jnp.max(top, axis=0, keepdims=True), jnp.int32) & 0x7F800000


def _combine(terms, get):
    acc = None
    for key, c in terms.items():
        v = get(key) if abs(c) == 1 else get(key) * abs(c)
        if acc is None:
            acc = v if c > 0 else -v
        else:
            acc = acc + v if c > 0 else acc - v
    return acc


def _kernel(x_hbm, w_hbm, b_hbm, o_hbm,
            xbuf, obuf, wbuf, bbuf, wt_ref, wc_ref, bb_ref, xs_ref, acc_ref,
            fsem, isem, osem, wsem):
    _, D, S = x_hbm.shape
    F = w_hbm.shape[1]
    H = F // 2
    NW = wt_ref.shape[0]
    NP = o_hbm.shape[0]
    RING = obuf.shape[0]
    G = 2 * S // _GROUP
    NC = S // _OCOLS
    NQ = 128 // 8 * NC
    QG = 2 * NQ // G
    first = [(sum(_FIRST[:j]), n) for j, n in enumerate(_FIRST)]

    def wcopy(j):
        rows = pl.ds(128 * j, min(128, D - 128 * j))
        return pltpu.make_async_copy(w_hbm.at[rows], wbuf.at[rows], wsem.at[j])

    def fcopy(h, j):
        cols = pl.ds(*first[j])
        return pltpu.make_async_copy(x_hbm.at[h, :, cols], xbuf.at[h, :, cols], fsem.at[2 * j + h])

    def icopy(m):
        both = pl.ds(2 * m, 2)
        return pltpu.make_async_copy(x_hbm.at[both], xbuf.at[both], isem.at[m])

    def ostart(m, slot, block):
        block = tuple(pl.ds(*b) for b in block)
        pltpu.make_async_copy(obuf.at[(slot,) + block], o_hbm.at[(m,) + block], osem.at[slot]).start()

    def owait(slot):
        pltpu.make_async_copy(obuf.at[slot], obuf.at[slot], osem.at[slot]).wait()

    def streams(r, c):
        return (0, 9), (8 * r, 8), (c, _OCOLS)

    def regular(q):
        return streams(q // NC, q % NC * _OCOLS)

    tail, pending = [], []
    for g in range(G):
        c = g // 2 * _GROUP
        for c0, n in _TAIL:
            if g % 2 and c + _GROUP == c0 + n:
                pending += [streams(r, cc) for r in range(16) for cc in range(c0, c0 + n, _OCOLS)]
        if c >= sum(_TAIL[-1]):
            batch = ((((0, 4), (0, 128)), ((4, 1), (0, 64))), (((4, 1), (64, 64)), ((5, 4), (0, 128))))
            pending += [rows + ((c, _GROUP),) for rows in batch[g % 2]]
        n = 2 * QG if g < G - 1 else len(pending)
        tail.append(pending[:n])
        pending = pending[n:]

    bcopy = pltpu.make_async_copy(b_hbm, bbuf, wsem.at[NW])
    bcopy.start()
    for j in range(NW):
        wcopy(j).start()
    for j in range(len(first)):
        lax.fori_loop(0, 2, lambda h, _: fcopy(h, j).start(), None)
    lax.fori_loop(1, NP, lambda m, _: icopy(m).start(), None)

    bcopy.wait()
    bias = bbuf[...].reshape(1, F).astype(jnp.float32)
    bb_ref[...] = jnp.broadcast_to(bias, (128, F)).T
    low = lax.broadcasted_iota(jnp.int32, (16, 128), 1) < 64
    expo, down, up = {}, {}, {}
    for j in range(NW):
        wcopy(j).wait()
        wp = _prune(wbuf[128 * j:min(128 * j + 128, D), :])
        if j == NW - 1:
            wp = jnp.concatenate([wp, wp], axis=0)
        wt = pltpu.bitcast(wp.T, jnp.int32)
        wt_ref[j] = wt
        if j < NW - 1:
            expo[j] = _max_exponent(wt)
            if j % 2 == 0:
                continue
            for t in (j - 1, j):
                shift = jnp.maximum(expo[t] - jnp.maximum(expo[j - 1], expo[j]), -64 << 23)
                down[t] = pltpu.bitcast((127 << 23) + shift, jnp.float32)
                up[t] = pltpu.bitcast((127 << 23) - shift, jnp.float32)
                xs_ref[pl.ds(128 * t, 128), :] = jnp.broadcast_to(down[t], (128, 128)).T
        for r in range(H // 16):
            wide = {}

            def get(key):
                i, t = key[0], _KROW[key[1]] // 128
                if (i, t) not in wide:
                    u = wt_ref[t, pl.ds(i * H // 2 + 8 * r, 8), :]
                    v = pltpu.bitcast(u, jnp.bfloat16).astype(jnp.float32)
                    wide[i, t] = v * up[t] if t in up else v
                return wide[i, t]

            for p, (_, ((w0, x0), (w1, x1))) in enumerate(_PASSES):
                if max(_KROW[k] // 128 | (k < 8) for _, k in (*w0, *w1)) == j:
                    v = jnp.where(low, _combine(w0, get), _combine(w1, get))
                    if len(x0) == len(x1) == 1:
                        t0, t1 = (_KROW[k] // 128 for k, _ in (*x0, *x1))
                        v = v * jnp.where(low, down[t0], down[t1])
                    wc_ref[p, pl.ds(16 * r, 16), :] = v.astype(wc_ref.dtype)

    def group(m, slot, h, o):
        wide = {}

        def raw(key):
            k, j = key
            return xbuf[2 * m + h, pl.ds(_KROW[k], 64), pl.ds(o + j * 128, 128)]

        def get(key):
            if key not in wide:
                v = raw(key).astype(jnp.float32)
                wide[key] = v * xs_ref[pl.ds(_KROW[key[0]], 64), :] if key[0] < 8 else v
            return wide[key]

        acc = [bb_ref[pl.ds(i * H, H), :] for i in (0, 0, 1, 1)]
        for p, (coef, products) in enumerate(_PASSES):
            if p and p % 4 == 0:
                for q in range(4):
                    acc_ref[q] = acc[q]
                acc = [acc_ref[q] for q in range(4)]
                wide.clear()
            if all(len(xt) == 1 for _, xt in products):
                xs = jnp.concatenate([raw(*xt) for _, xt in products], axis=0)
            else:
                xs = jnp.concatenate([_combine(xt, get) for _, xt in products], axis=0)
            y = jnp.dot(wc_ref[p], xs.astype(wc_ref.dtype), preferred_element_type=jnp.float32)
            for q, c in enumerate(coef):
                if c == -1:
                    acc[q] = acc[q] - y
                elif c:
                    acc[q] = acc[q] + (y if c == 1 else y + y)
        for q in range(4):
            out = acc[q].astype(obuf.dtype)
            r0 = h * F + q // 2 * H
            cuts = sorted({r0, r0 + H} | set(range(pl.cdiv(r0, 128) * 128, r0 + H, 128)))
            for lo, hi in zip(cuts[:-1], cuts[1:]):
                obuf[slot, lo // 128, pl.ds(lo % 128, hi - lo), pl.ds(o + q % 2 * 128, 128)] = (
                    out[lo - r0:hi - r0])

    def wrap(s):
        return jnp.where(s >= RING, s - RING, s)

    def pair(m, slot):
        def only_at(step, n, block):
            pl.when(m == step)(lambda: ostart(n, n % RING, block))

        pl.when(m > 0)(lambda: icopy(m).wait())
        pl.when(m >= RING)(lambda: owait(slot))
        done = [jnp.clip(2 * m - NP + d, 0, NP - 1) for d in range(3)]
        for g in range(G):
            h, o = g % 2, g // 2 * _GROUP
            for j in range(len(first)):
                if first[j][0] == o:
                    pl.when(m == 0)(lambda: fcopy(h, j).wait())
            if g == 0:
                for q in range(QG, _LEAD):
                    only_at(NP - 1, NP - 2, regular(q))
            group(m, slot, h, o)
            for q in range(_LEAD):
                if g == max(_START, G - pl.cdiv(_LEAD - q, QG)):
                    only_at(NP // 2 - 1, 0, regular(q))
            for e in range(QG):
                d, q = divmod(_LEAD + QG * g + e, NQ)
                finished = jnp.logical_and(m >= NP // 2, m < NP - d)
                pl.when(finished)(lambda: ostart(done[d], wrap(done[d]), regular(q)))
            for block in tail[g]:
                only_at(NP - 1, NP - 1, block)
        for q in range(QG):
            only_at(NP - 2, NP - 2, regular(q))
        return wrap(slot + 1)

    lax.fori_loop(0, NP, pair, 0)
    for m in range(NP - RING, NP):
        owait(m % RING)


@jax.jit
def pallas_standalone__structured_sparse_n_m__ragged_kernel(
    x: jax.Array,
    w: jax.Array,
    b: jax.Array,
):
    B, S, D = x.shape
    F = w.shape[1]
    tiles = pl.cdiv(D, 128)
    ring = B // 4 + 1
    xt = jnp.transpose(x, (0, 2, 1))
    out = pl.pallas_call(
        _kernel,
        in_specs=[pl.BlockSpec(memory_space=pl.ANY)] * 3,
        out_specs=pl.BlockSpec(memory_space=pl.ANY),
        out_shape=jax.ShapeDtypeStruct((B // 2, 2 * F // 128, 128, S), x.dtype),
        scratch_shapes=[
            pltpu.VMEM((B, D, S), x.dtype),
            pltpu.VMEM((ring, 2 * F // 128, 128, S), x.dtype),
            pltpu.VMEM((D, F), w.dtype),
            pltpu.VMEM((F,), b.dtype),
            pltpu.VMEM((tiles, F // 2, 128), jnp.int32),
            pltpu.VMEM((len(_PASSES), F // 2, 128), jnp.bfloat16),
            pltpu.VMEM((F, 128), jnp.float32),
            pltpu.VMEM((D // 128 * 128, 128), jnp.float32),
            pltpu.VMEM((4, F // 2, 128), jnp.float32),
            pltpu.SemaphoreType.DMA((2 * len(_FIRST),)),
            pltpu.SemaphoreType.DMA((B // 2,)),
            pltpu.SemaphoreType.DMA((ring,)),
            pltpu.SemaphoreType.DMA((tiles + 1,)),
        ],
        compiler_params=pltpu.CompilerParams(
            vmem_limit_bytes=127 * 1024 * 1024,
            disable_bounds_checks=True,
            disable_semaphore_checks=True,
            flags={"XLA_TPU_RESCHEDULE_DMA_DONES": True},
        ),
    )(xt, w, b)
    return jnp.transpose(out.reshape(B, F, S), (0, 2, 1))
```
